```python
import os as _os
_os.environ.setdefault("JAX_PLATFORMS", "cpu")
import jax
import jax.numpy as jnp

def _softmax(x, axis=-1):
    return jax.nn.softmax(x, axis=axis)
def _gelu(x):
    return jax.nn.gelu(x, approximate=True)
def _silu(x):
    return jax.nn.silu(x)
def _sigmoid(x):
    return jax.nn.sigmoid(x)
def _layernorm(x, axis=-1, eps=1e-5):
    m = jnp.mean(x, axis=axis, keepdims=True)
    v = jnp.var(x, axis=axis, keepdims=True)
    return (x - m) / jnp.sqrt(v + eps)
def _scatter_add(tgt, idx, src, axis=0):
    return tgt.at[idx].add(src)
def _segment_sum(src, seg, n):
    return jax.ops.segment_sum(src, seg, n)
class _Rng:
    def __init__(self, key):
        self._k = key
    def _next(self):
        self._k, sub = jax.random.split(self._k)
        return sub
    def normal(self, shape):
        return jax.random.normal(self._next(), shape, dtype=jnp.bfloat16)
    def randint(self, lo, hi, shape):
        return jax.random.randint(self._next(), shape, lo, hi, dtype=jnp.int32)
    def uniform(self, shape, lo=0.0, hi=1.0):
        return jax.random.uniform(self._next(), shape, jnp.bfloat16, lo, hi)
    def permutation(self, n):
        return jax.random.permutation(self._next(), n)


kernel_name = 'sequential_preLN__sliding_local_dilated__dense_activation_mish__prompt'

def setup_inputs():
    _rng = _Rng(jax.random.key(int.from_bytes(__import__("os").urandom(4), "little")))
    _w = (lambda a: (lambda t: t.astype(jnp.bfloat16) if jnp.issubdtype(t.dtype, jnp.floating) else t)(jnp.asarray(a)))
    def _A_setup():
        B, S, D = 1, 2048, 512
        return {
            "x": _w((lambda *s: _rng.normal(s) * 0.05)(B, S, D)),
            "wqkv": _w((lambda *s: _rng.normal(s) * 0.05)(D, 3 * D)),
            "wo": _w((lambda *s: _rng.normal(s) * 0.05)(D, D)),
        }
    _A_in = _A_setup()

    def _B_setup():
        B, S, D, F = 1, 2048, 512, 1376
        return {
            "x": _w((lambda *s: _rng.normal(s) * 0.05)(B, S, D)),
            "w1": _w((lambda *s: _rng.normal(s) * 1.6)(D, F) * (D ** -0.5)),
            "b1": _w((lambda *s: _rng.normal(s) * 0.1)(F)),
            "w2": _w((lambda *s: _rng.normal(s) * 0.1)(F, D) * (F ** -0.5)),
        }
    _B_in = _B_setup()

    return {
        "A_x": _A_in["x"],
        "A_wqkv": _A_in["wqkv"],
        "A_wo": _A_in["wo"],
        "B_x": _B_in["x"],
        "B_w1": _B_in["w1"],
        "B_b1": _B_in["b1"],
        "B_w2": _B_in["w2"],
    }

def reference(A_x, A_wqkv, A_wo, B_x, B_w1, B_b1, B_w2):
    def _A_ref(x, wqkv, wo):
        B, S, D = x.shape
        H = 32; Dh = D // H
        W, dil = 8, 2
        qkv = (lambda x, *d: x.transpose(*d))((x @ wqkv).reshape(B, S, 3, H, Dh), 2, 0, 3, 1, 4)
        q, k, v = qkv[0], qkv[1], qkv[2]
        scale = Dh ** -0.5
        pos = jnp.arange(S)
        off = jnp.arange(W) * dil
        idx = pos[:, None] - off[None, :]
        mask = idx >= 0
        idx_c = jnp.where(mask, idx, 0).reshape(-1)
        kg = k[:, :, idx_c, :].reshape(B, H, S, W, Dh)
        vg = v[:, :, idx_c, :].reshape(B, H, S, W, Dh)
        logits = jnp.einsum("bhsd,bhswd->bhsw", q, kg) * scale
        logits = jnp.where(mask[None, None, :, :], logits, -1e9)
        attn = _softmax(logits, axis=-1)
        o = jnp.einsum("bhsw,bhswd->bhsd", attn, vg)
        return (lambda x, *d: x.transpose(*d))(o, 0, 2, 1, 3).reshape(B, S, D) @ wo

    def _B_ref(x, w1, b1, w2):
        h = jnp.einsum("bsd,df->bsf", x, w1) + b1
        sp = jnp.log1p(jnp.exp(-jnp.abs(h))) + jnp.where(h > 0, h, jnp.zeros_like(h))
        act = h * jnp.tanh(sp)
        return jnp.einsum("bsf,fd->bsd", act, w2)

    x = A_x
    h = x + _A_ref(_layernorm(x, axis=-1), A_wqkv, A_wo)
    h2 = h + _B_ref(_layernorm(h, axis=-1), B_w1, B_b1, B_w2)
    return h2
```

```python
import jax
import jax.numpy as jnp
from jax import lax
import jax.experimental.pallas as pl
import jax.experimental.pallas.tpu as pltpu

S, D, F = 2048, 512, 1376
W, DIL = 8, 2
FP = 1408
NF = FP // 128
TM = 256
NT = S // TM
G = TM // 8
HALO = 16
LAG = 2
PACE = 4
SCALE2 = 0.25 * 1.4426950408889634
MASKED2 = -1e9 * 1.4426950408889634
NT_DIMS = (((1,), (1,)), ((), ()))
BF, U32, F32 = jnp.bfloat16, jnp.uint32, jnp.float32


def _recip(x):
    r = pl.reciprocal(x, approx=True)
    return r * (2.0 - x * r)


def _layernorm(hs):
    s = (hs[0] + hs[1]) + (hs[2] + hs[3])
    m = jnp.sum(s, axis=-1, keepdims=True) * (1.0 / D)
    xc = [h - m for h in hs]
    sq = (xc[0] * xc[0] + xc[1] * xc[1]) + (xc[2] * xc[2] + xc[3] * xc[3])
    v = jnp.sum(sq, axis=-1, keepdims=True) * (1.0 / D)
    r = lax.rsqrt(v + 1e-5)
    return [c * r for c in xc]


def _as_bf16(words):
    return pltpu.bitcast(words, BF)


def _weave(a, b):
    keyed = [(n / len(a), 0, n) for n in range(len(a))] + [((n + 0.5) / len(b), 1, n) for n in range(len(b))]
    keyed.sort()
    return [(a, b)[li][n] for _, li, n in keyed]


def _kernel(x_hbm, wqkv_hbm, wo_hbm, w1t_hbm, b1_hbm, w2_hbm, o_hbm,
            x_vm, wq_vm, wkv32, tr_scr, wkvp32, wo32, wop32, w1_vm, w2_vm, wqt,
            xln, q_scr, k_scr, v_scr, o_scr, h_scr, hln, act, out_vm, b1_scr, b1_vm, sem):

    def cp(src, dst, k):
        return pltpu.make_async_copy(src, dst, sem.at[k])

    wqkv32_hbm = wqkv_hbm.bitcast(U32)
    wo32_hbm = wo_hbm.bitcast(U32)

    def dma_x(lo, n, k):
        return [cp(x_hbm.at[0, pl.ds(lo, n), :], x_vm.at[pl.ds(lo, n), :], k)]

    dma = dict(
        x0=lambda: dma_x(0, TM, 0),
        x1=lambda: dma_x(TM, TM, 3),
        x2=lambda: dma_x(2 * TM, TM, 3),
        xr=lambda: dma_x(3 * TM, S - 3 * TM, 2),
        qa=lambda: [cp(wqkv_hbm.at[:, pl.ds(0, 256)], wq_vm.at[:, pl.ds(0, 256)], 1)],
        qb=lambda: [cp(wqkv_hbm.at[:, pl.ds(256, 256)], wq_vm.at[:, pl.ds(256, 256)], 2)],
        k=lambda: [cp(wqkv32_hbm.at[:, pl.ds(512, 512)], wkv32.at[0], 0)],
        v=lambda: [cp(wqkv32_hbm.at[:, pl.ds(1024, 512)], wkv32.at[1], 1)],
        wo=lambda: [cp(wo32_hbm.at[:, pl.ds(j * 128, 128)], wo32.at[j, pl.ds(0, D // 2), :], 2) for j in range(4)],
        w1=lambda: [cp(w1t_hbm.at[:, pl.ds(j * 128, 128)], w1_vm.at[j, pl.ds(0, F), :], 0) for j in range(4)],
        w2=lambda: [cp(w2_hbm.at[:, pl.ds(j * 128, 128)], w2_vm.at[j, pl.ds(0, F), :], 1) for j in range(4)],
        b1=lambda: [cp(b1_hbm, b1_vm, 4)],
    )

    def start(*names):
        for nm in names:
            for c in dma[nm]():
                c.start()

    def wait(*names):
        for nm in names:
            for c in dma[nm]():
                c.wait()

    w1w, w2w, wqtw = w1_vm.bitcast(U32), w2_vm.bitcast(U32), wqt.bitcast(U32)
    xlnw, ow, hlnw, actw = xln.bitcast(U32), o_scr.bitcast(U32), hln.bitcast(U32), act.bitcast(U32)

    r_ = lax.broadcasted_iota(jnp.int32, (128, 128), 0)
    f_ = lax.broadcasted_iota(jnp.int32, (128, 128), 1)
    PERM = (f_ == ((r_ & 7) << 4) + (r_ >> 3)).astype(F32).astype(BF)
    for j in range(4):
        w1_vm[j, F:FP, :] = jnp.zeros((FP - F, 128), BF)
        w2_vm[j, F:FP, :] = jnp.zeros((FP - F, 128), BF)

    def prep_b1():
        b1 = b1_vm[...].astype(F32).reshape(1, F)
        b1 = jnp.concatenate([b1, jnp.zeros((1, FP - F), F32)], axis=1)
        for j in range(NF):
            b1_scr[j] = jnp.broadcast_to(b1[:, j * 128:(j + 1) * 128], (8, 128))

    q_part = {}

    def prep_q(half):
        for t in (2 * half, 2 * half + 1):
            w = wq_vm[:, t * 128:(t + 1) * 128]
            q_part[t] = lax.dot_general(PERM, w, NT_DIMS, preferred_element_type=F32).reshape(16, 8, D)
        if half == 1:
            full = jnp.stack([q_part[t] for t in range(4)], axis=1).reshape(D, D)
            for kk in range(4):
                wqt[kk] = full[:, kk * 128:(kk + 1) * 128].astype(BF)

    def prep_kv(p):
        for rb in range(2):
            for t in range(4):
                tr_scr[p, rb, t * 128:(t + 1) * 128, :] = wkv32[p, rb * 128:(rb + 1) * 128, t * 128:(t + 1) * 128].T
        for jp in range(4):
            for rb in range(2):
                tile = jnp.concatenate([tr_scr[p, rb, pl.ds(4 * jp + c, 32, stride=16), :] for c in range(4)], axis=0)
                wkvp32[p, jp, rb * 128:(rb + 1) * 128, :] = tile.T

    def prep_wo():
        for jn in range(4):
            for u in range(2):
                for dp in range(8):
                    e = wo32[jn, pl.ds(128 * u + dp, 8, stride=16), :]
                    o = wo32[jn, pl.ds(128 * u + dp + 8, 8, stride=16), :]
                    wop32[jn, pl.ds((2 * dp) * 16 + 8 * u, 8), :] = (e & jnp.uint32(0xFFFF)) | (o << 16)
                    wop32[jn, pl.ds((2 * dp + 1) * 16 + 8 * u, 8), :] = (e >> 16) | (o & jnp.uint32(0xFFFF0000))

    def rows(t, r, n, extra=0):
        base, c = t
        off = c * TM + r + extra
        return pl.ds(off, n) if base is None else pl.ds(base[0] + off, n)

    def wrows(t, r, n):
        base, c = t
        off = (c * TM + r) // 2
        return pl.ds(off, n // 2) if base is None else pl.ds(base[1] + off, n // 2)

    def first(t):
        return t[0] is None and t[1] == 0

    def ln1(t):
        for r in range(0, TM, 16):
            x = x_vm[rows(t, r, 16), :].astype(F32)
            y = _layernorm([x[:, kk * 128:(kk + 1) * 128] for kk in range(4)])
            for kk in range(4):
                xln[kk, rows(t, r, 16), :] = y[kk].astype(BF)

    def qkv(t, j):
        lhs = jnp.concatenate([_as_bf16(xlnw[kk, wrows(t, 0, TM), :]) for kk in range(4)], axis=1)
        p, jj = divmod(j, 4)
        if p == 0:
            rhs = jnp.concatenate([_as_bf16(wqtw[kk, j * 64:(j + 1) * 64, :]) for kk in range(4)], axis=1)
            q_scr[jj, rows(t, 0, TM), :] = lax.dot_general(lhs, rhs, NT_DIMS, preferred_element_type=F32)
            return
        res = jnp.dot(lhs, _as_bf16(wkvp32[p - 1, jj]), preferred_element_type=F32)
        scr = k_scr if p == 1 else v_scr
        scr[jj, rows(t, 0, TM, HALO), :] = res
        if first(t):
            scr[jj, 0:HALO, :] = jnp.broadcast_to(res[0:1, :], (HALO, 128))

    sums, gates, pending = {}, {}, {}

    def attn_logits(t, g):
        q = [q_scr[j, rows(t, g * 8, 8), :] for j in range(4)]
        if (t[1], g - PACE) in sums:
            pace = sums.pop((t[1], g - PACE))
            cq = jnp.where(pace < 0.0, pace, SCALE2)
        elif gates.get("on") in gates:
            pace = gates[gates["on"]]
            cq = jnp.where(pace < 0.0, pace, SCALE2)
        else:
            cq = SCALE2
        q = [q_ * cq for q_ in q]
        parts = []
        for w in range(W):
            acc = None
            for j in range(4):
                pr = q[j] * k_scr[j, rows(t, g * 8, 8, HALO - DIL * w), :]
                acc = pr if acc is None else acc + pr
            parts.append(acc)
        return parts, [[pltpu.roll(p, sh, 1) for sh in (32, 64, 96)] for p in parts]

    def attn_values(t, g, state):
        parts, rolled = state
        logits = []
        for w in range(W):
            l = (parts[w] + rolled[w][0]) + (rolled[w][1] + rolled[w][2])
            if first(t) and w > 0 and g * 8 < DIL * w:
                row = g * 8 + lax.broadcasted_iota(jnp.int32, (8, 128), 0)
                l = jnp.where(row >= DIL * w, l, MASKED2)
            logits.append(l)
        m = jnp.maximum(jnp.maximum(jnp.maximum(logits[0], logits[1]), jnp.maximum(logits[2], logits[3])),
                        jnp.maximum(jnp.maximum(logits[4], logits[5]), jnp.maximum(logits[6], logits[7])))
        pw = [jnp.exp2(l - m) for l in logits]
        den = ((pw[0] + pw[1]) + (pw[2] + pw[3])) + ((pw[4] + pw[5]) + (pw[6] + pw[7]))
        sums[(t[1], g)] = den
        inv = _recip(den)
        outs = []
        for j in range(4):
            acc = None
            for w in range(W):
                pr = pw[w] * v_scr[j, rows(t, g * 8, 8, HALO - DIL * w), :]
                acc = pr if acc is None else acc + pr
            outs.append(acc * inv)
        return outs

    def attn(t, m):
        c = t[1]
        if m < G:
            pending[(c, m)] = attn_logits(t, m)
        g = m - LAG
        if g >= 0:
            pending[(c, g, "o")] = attn_values(t, g, pending.pop((c, g)))
            if g % 2 == 1:
                a, b = pending.pop((c, g - 1, "o")), pending.pop((c, g, "o"))
                for j in range(4):
                    o_scr[j, rows(t, (g - 1) * 8, 16), :] = jnp.concatenate([a[j], b[j]], axis=0).astype(BF)

    def proj(t, jn):
        lhs = jnp.concatenate([_as_bf16(ow[kk, wrows(t, 0, TM), :]) for kk in range(4)], axis=1)
        res = jnp.dot(lhs, _as_bf16(wop32[jn]), preferred_element_type=F32)
        h_scr[jn, rows(t, 0, TM), :] = res + x_vm[rows(t, 0, TM), jn * 128:(jn + 1) * 128].astype(F32)

    def ln2(t):
        for r in range(0, TM, 16):
            y = _layernorm([h_scr[jn, rows(t, r, 16), :] for jn in range(4)])
            for kk in range(4):
                hln[kk, rows(t, r, 16), :] = y[kk].astype(BF)

    def up(t, j):
        lhs = jnp.concatenate([_as_bf16(hlnw[kk, wrows(t, 0, TM), :]) for kk in range(4)], axis=1)
        rhs = jnp.concatenate([_as_bf16(w1w[kk, j * 64:(j + 1) * 64, :]) for kk in range(4)], axis=1)
        pre = lax.dot_general(lhs, rhs, NT_DIMS, preferred_element_type=F32)
        pre = pre + jnp.tile(b1_scr[j], (TM // 8, 1))
        e = jnp.exp(jnp.minimum(pre, 20.0))
        n = e * (e + 2.0)
        den = n + 2.0
        gates[j] = den[0:8, :]
        act[j, rows(t, 0, TM), :] = (pre * n * _recip(den)).astype(BF)

    def down(t, jn):
        lhs = jnp.concatenate([_as_bf16(actw[j, wrows(t, 0, TM), :]) for j in range(NF)], axis=1)
        res = jnp.dot(lhs, _as_bf16(w2w[jn]), preferred_element_type=F32)
        out_vm[rows(t, 0, TM), jn * 128:(jn + 1) * 128] = (res + h_scr[jn, rows(t, 0, TM), :]).astype(BF)

    def out_tile(t):
        return cp(out_vm.at[rows(t, 0, TM), :], o_hbm.at[0, rows(t, 0, TM), :], 3)

    def out_cols(t, jn):
        return cp(out_vm.at[rows(t, 0, TM), pl.ds(jn * 128, 128)], o_hbm.at[0, rows(t, 0, TM), pl.ds(jn * 128, 128)], 3)

    def each(fn, t, lo, hi):
        return [lambda i=i: fn(t, i) for i in range(lo, hi + 1)]

    def run(thunks):
        for th in thunks:
            th()

    def weave(a, b):
        run(_weave(a, b))

    LAST = G + LAG - 1
    T = [(None, i) for i in range(NT)]

    start("x0", "qa")
    start("qb", "x1", "b1")
    wait("x0", "qa")
    start("k", "v")
    ln1(T[0])
    prep_q(0)
    wait("qb")
    prep_q(1)
    wait("x1")
    ln1(T[1])
    run(each(qkv, T[0], 0, 3))
    wait("k")
    start("wo", "x2")
    prep_kv(0)
    run(each(qkv, T[1], 0, 3))
    run(each(qkv, T[0], 4, 4))
    wait("v")
    start("w1")
    prep_kv(1)
    run(each(qkv, T[0], 5, 7))
    run(each(qkv, T[1], 4, 5))
    run(each(qkv, T[0], 8, 11))
    weave(each(qkv, T[1], 6, 8), each(attn, T[0], 0, 25))
    wait("wo", "x2", "b1", "w1")
    start("w2", "xr")
    prep_wo()
    prep_b1()
    ln1(T[2])
    weave(each(qkv, T[1], 9, 11), each(attn, T[0], 26, LAST))
    run(each(proj, T[0], 0, 3))
    run(each(qkv, T[2], 0, 3))
    ln2(T[0])
    run(each(up, T[0], 0, NF - 1))
    weave(each(qkv, T[2], 4, 7), each(attn, T[1], 0, 6))
    wait("w2", "xr")
    weave(each(qkv, T[2], 8, 11), each(attn, T[1], 7, 14))
    weave(each(down, T[0], 0, 3), each(attn, T[1], 15, LAST))
    ln1(T[3])
    out_tile(T[0]).start()

    def step(r, carry):
        sums.clear(); gates.clear(); pending.clear()
        s = 1 + r
        base = (pl.multiple_of(s * TM, TM), pl.multiple_of(s * (TM // 2), TM // 2))
        t0, t1, t2, t3 = (base, 0), (base, 1), (base, 2), (base, 3)
        run(each(proj, t0, 0, 3))
        run(each(qkv, t2, 0, 3))
        ln2(t0)
        run(each(up, t0, 0, NF - 1))
        weave(each(qkv, t2, 4, 11), each(attn, t1, 0, 14))
        weave(each(down, t0, 0, 3), each(attn, t1, 15, LAST))
        ln1(t3)
        out_tile(t0).start()
        sums.clear(); gates.clear(); pending.clear()
        return carry

    lax.fori_loop(0, 4, step, 0)

    run(each(proj, T[5], 0, 3))
    run(each(qkv, T[7], 0, 3))
    ln2(T[5])
    run(each(up, T[5], 0, NF - 1))
    weave(each(qkv, T[7], 4, 7), each(attn, T[6], 0, 7))
    weave(each(down, T[5], 0, 3), each(attn, T[6], 8, LAST))
    out_tile(T[5]).start()

    run(each(proj, T[6], 0, 3))
    run(each(qkv, T[7], 8, 11))
    ln2(T[6])
    run(each(up, T[6], 0, NF - 1))
    gates["on"] = NF - 1
    weave(each(down, T[6], 0, 2), each(attn, T[7], 0, LAST))
    gates["on"] = None

    run(each(proj, T[7], 0, 3))
    down(T[6], 3)
    ln2(T[7])
    out_tile(T[6]).start()
    run(each(up, T[7], 0, NF - 1))
    for jn in range(4):
        down(T[7], jn)
        out_cols(T[7], jn).start()

    for i in range(NT - 1):
        out_tile(T[i]).wait()
    for jn in range(4):
        out_cols(T[7], jn).wait()


@jax.jit
def pallas_sequential_preLN__sliding_local_dilated__dense_activation_mish__prompt_kernel(
    A_x: jax.Array,
    A_wqkv: jax.Array,
    A_wo: jax.Array,
    B_x: jax.Array,
    B_w1: jax.Array,
    B_b1: jax.Array,
    B_w2: jax.Array,
):
    del B_x
    hbm = pl.BlockSpec(memory_space=pltpu.HBM)
    return pl.pallas_call(
        _kernel,
        in_specs=[hbm] * 6,
        out_specs=hbm,
        out_shape=jax.ShapeDtypeStruct((1, S, D), BF),
        scratch_shapes=[
            pltpu.VMEM((S, D), BF),
            pltpu.VMEM((D, D), BF),
            pltpu.VMEM((2, D // 2, D), U32),
            pltpu.VMEM((2, 2, D + 16, 128), U32),
            pltpu.VMEM((2, 4, D // 2, 128), U32),
            pltpu.VMEM((4, D // 2 + 16, 128), U32),
            pltpu.VMEM((4, D // 2, 128), U32),
            pltpu.VMEM((4, FP, 128), BF),
            pltpu.VMEM((4, FP, 128), BF),
            pltpu.VMEM((4, D, 128), BF),
            pltpu.VMEM((4, S, 128), BF),
            pltpu.VMEM((4, S, 128), F32),
            pltpu.VMEM((4, HALO + S, 128), F32),
            pltpu.VMEM((4, HALO + S, 128), F32),
            pltpu.VMEM((4, S, 128), BF),
            pltpu.VMEM((4, S, 128), F32),
            pltpu.VMEM((4, S, 128), BF),
            pltpu.VMEM((NF, S, 128), BF),
            pltpu.VMEM((S, D), BF),
            pltpu.VMEM((NF, 8, 128), F32),
            pltpu.VMEM((F,), BF),
            pltpu.SemaphoreType.DMA((5,)),
        ],
        compiler_params=pltpu.CompilerParams(vmem_limit_bytes=64 << 20),
        name="preln_dilated_attn_mish_ffn",
    )(A_x, A_wqkv, A_wo, B_w1.T, B_b1, B_w2)
```

```python
import jax
import jax.numpy as jnp
from jax import lax
import jax.experimental.pallas as pl
import jax.experimental.pallas.tpu as pltpu

S, D, F = 2048, 512, 1376
W, DIL = 8, 2
FP = 1408
NF = FP // 128
TM = 256
NT = S // TM
G = TM // 8
HALO = 16
LAG = 2
PACE = 4
SCALE2 = 0.25 * 1.4426950408889634
MASKED2 = -1e9 * 1.4426950408889634
NT_DIMS = (((1,), (1,)), ((), ()))
BF, U32, F32 = jnp.bfloat16, jnp.uint32, jnp.float32


def _recip(x):
    r = pl.reciprocal(x, approx=True)
    return r * (2.0 - x * r)


def _layernorm(hs):
    s = (hs[0] + hs[1]) + (hs[2] + hs[3])
    m = jnp.sum(s, axis=-1, keepdims=True) * (1.0 / D)
    xc = [h - m for h in hs]
    sq = (xc[0] * xc[0] + xc[1] * xc[1]) + (xc[2] * xc[2] + xc[3] * xc[3])
    v = jnp.sum(sq, axis=-1, keepdims=True) * (1.0 / D)
    r = lax.rsqrt(v + 1e-5)
    return [c * r for c in xc]


def _as_bf16(words):
    return pltpu.bitcast(words, BF)


def _weave(a, b):
    keyed = [(n / len(a), 0, n) for n in range(len(a))] + [((n + 0.5) / len(b), 1, n) for n in range(len(b))]
    keyed.sort()
    return [(a, b)[li][n] for _, li, n in keyed]


def _kernel(x_hbm, wqkv_hbm, wo_hbm, w1t_hbm, b1_hbm, w2_hbm, o_hbm,
            x_vm, wq_vm, wkv32, tr_scr, wkvp32, wo32, wop32, w1_vm, w2_vm, wqt,
            xln, q_scr, k_scr, v_scr, o_scr, h_scr, hln, act, out_vm, b1_scr, b1_vm, sem):

    def after(v):
        return (jnp.max(jnp.abs(v)) < -1.0).astype(jnp.int32)

    def cp(src, dst, k, z=None):
        return pltpu.make_async_copy(src, dst, sem.at[k if z is None else k + z])

    wqkv32_hbm = wqkv_hbm.bitcast(U32)
    wo32_hbm = wo_hbm.bitcast(U32)

    def dma_x(lo, n, k, z):
        return [cp(x_hbm.at[0, pl.ds(lo, n), :], x_vm.at[pl.ds(lo, n), :], k, z)]

    SA, SB, SC, SK, SV = range(5)
    dma = dict(
        x0=lambda z: dma_x(0, TM, SA, z),
        qa=lambda z: [cp(wqkv_hbm.at[:, pl.ds(0, 256)], wq_vm.at[:, pl.ds(0, 256)], SA, z)],
        qb=lambda z: [cp(wqkv_hbm.at[:, pl.ds(256, 256)], wq_vm.at[:, pl.ds(256, 256)], SB, z)],
        x1=lambda z: dma_x(TM, TM, SC, z),
        b1=lambda z: [cp(b1_hbm, b1_vm, SC, z)],
        k=lambda z: [cp(wqkv32_hbm.at[:, pl.ds(512, 512)], wkv32.at[0], SK, z)],
        v=lambda z: [cp(wqkv32_hbm.at[:, pl.ds(1024, 512)], wkv32.at[1], SV, z)],
        wo=lambda z: [cp(wo32_hbm.at[:, pl.ds(j * 128, 128)], wo32.at[j, pl.ds(0, D // 2), :], SA, z) for j in range(4)],
        x2=lambda z: dma_x(2 * TM, TM, SA, z),
        w1=lambda z: [cp(w1t_hbm.at[:, pl.ds(j * 128, 128)], w1_vm.at[j, pl.ds(0, F), :], SK, z) for j in range(4)],
        w2=lambda z: [cp(w2_hbm.at[:, pl.ds(j * 128, 128)], w2_vm.at[j, pl.ds(0, F), :], SV, z) for j in range(4)],
        xr=lambda z: dma_x(3 * TM, S - 3 * TM, SV, z),
    )
    OUT_SEM = SB

    def start(*names, z=None):
        for nm in names:
            for c in dma[nm](z):
                c.start()

    def wait(*names, z=None):
        for nm in names:
            for c in dma[nm](z):
                c.wait()

    w1w, w2w, wqtw = w1_vm.bitcast(U32), w2_vm.bitcast(U32), wqt.bitcast(U32)
    xlnw, ow, hlnw, actw = xln.bitcast(U32), o_scr.bitcast(U32), hln.bitcast(U32), act.bitcast(U32)

    r_ = lax.broadcasted_iota(jnp.int32, (128, 128), 0)
    f_ = lax.broadcasted_iota(jnp.int32, (128, 128), 1)
    PERM = (f_ == ((r_ & 7) << 4) + (r_ >> 3)).astype(F32).astype(BF)
    for j in range(4):
        w1_vm[j, F:FP, :] = jnp.zeros((FP - F, 128), BF)
        w2_vm[j, F:FP, :] = jnp.zeros((FP - F, 128), BF)

    def prep_b1():
        b1 = b1_vm[...].astype(F32).reshape(1, F)
        b1 = jnp.concatenate([b1, jnp.zeros((1, FP - F), F32)], axis=1)
        for j in range(NF):
            b1_scr[j] = jnp.broadcast_to(b1[:, j * 128:(j + 1) * 128], (8, 128))

    q_part, seen = {}, {}

    def prep_q(half):
        for t in (2 * half, 2 * half + 1):
            w = wq_vm[:, t * 128:(t + 1) * 128]
            q_part[t] = lax.dot_general(PERM, w, NT_DIMS, preferred_element_type=F32).reshape(16, 8, D)
        if half == 1:
            full = jnp.stack([q_part[t] for t in range(4)], axis=1).reshape(D, D)
            seen["wq"] = full[0:8, 0:128]
            for kk in range(4):
                wqt[kk] = full[:, kk * 128:(kk + 1) * 128].astype(BF)

    def prep_kv(p):
        for rb in range(2):
            for t in range(4):
                tr_scr[p, rb, t * 128:(t + 1) * 128, :] = wkv32[p, rb * 128:(rb + 1) * 128, t * 128:(t + 1) * 128].T
        for jp in range(4):
            for rb in range(2):
                tile = jnp.concatenate([tr_scr[p, rb, pl.ds(4 * jp + c, 32, stride=16), :] for c in range(4)], axis=0)
                wkvp32[p, jp, rb * 128:(rb + 1) * 128, :] = tile.T

    def prep_wo():
        for jn in range(4):
            for u in range(2):
                for dp in range(8):
                    e = wo32[jn, pl.ds(128 * u + dp, 8, stride=16), :]
                    o = wo32[jn, pl.ds(128 * u + dp + 8, 8, stride=16), :]
                    wop32[jn, pl.ds((2 * dp) * 16 + 8 * u, 8), :] = (e & jnp.uint32(0xFFFF)) | (o << 16)
                    wop32[jn, pl.ds((2 * dp + 1) * 16 + 8 * u, 8), :] = (e >> 16) | (o & jnp.uint32(0xFFFF0000))

    def rows(t, r, n, extra=0):
        base, c = t
        off = c * TM + r + extra
        return pl.ds(off, n) if base is None else pl.ds(base[0] + off, n)

    def wrows(t, r, n):
        base, c = t
        off = (c * TM + r) // 2
        return pl.ds(off, n // 2) if base is None else pl.ds(base[1] + off, n // 2)

    def first(t):
        return t[0] is None and t[1] == 0

    def ln1(t):
        for r in range(0, TM, 16):
            x = x_vm[rows(t, r, 16), :].astype(F32)
            y = _layernorm([x[:, kk * 128:(kk + 1) * 128] for kk in range(4)])
            for kk in range(4):
                xln[kk, rows(t, r, 16), :] = y[kk].astype(BF)
            seen["ln1", t[1]] = y[3][0:8, :]

    def qkv(t, j):
        lhs = jnp.concatenate([_as_bf16(xlnw[kk, wrows(t, 0, TM), :]) for kk in range(4)], axis=1)
        p, jj = divmod(j, 4)
        if p == 0:
            rhs = jnp.concatenate([_as_bf16(wqtw[kk, j * 64:(j + 1) * 64, :]) for kk in range(4)], axis=1)
            res = lax.dot_general(lhs, rhs, NT_DIMS, preferred_element_type=F32)
            seen["qkv", t[1], j] = res[0:8, :]
            q_scr[jj, rows(t, 0, TM), :] = res
            return
        res = jnp.dot(lhs, _as_bf16(wkvp32[p - 1, jj]), preferred_element_type=F32)
        seen["qkv", t[1], j] = res[0:8, :]
        scr = k_scr if p == 1 else v_scr
        scr[jj, rows(t, 0, TM, HALO), :] = res
        if first(t):
            scr[jj, 0:HALO, :] = jnp.broadcast_to(res[0:1, :], (HALO, 128))

    sums, gates, pending = {}, {}, {}

    def attn_logits(t, g):
        q = [q_scr[j, rows(t, g * 8, 8), :] for j in range(4)]
        if (t[1], g - PACE) in sums:
            pace = sums.pop((t[1], g - PACE))
            cq = jnp.where(pace < 0.0, pace, SCALE2)
        elif gates.get("on") in gates:
            pace = gates[gates["on"]]
            cq = jnp.where(pace < 0.0, pace, SCALE2)
        else:
            cq = SCALE2
        q = [q_ * cq for q_ in q]
        parts = []
        for w in range(W):
            acc = None
            for j in range(4):
                pr = q[j] * k_scr[j, rows(t, g * 8, 8, HALO - DIL * w), :]
                acc = pr if acc is None else acc + pr
            parts.append(acc)
        return parts, [[pltpu.roll(p, sh, 1) for sh in (32, 64, 96)] for p in parts]

    def attn_values(t, g, state):
        parts, rolled = state
        logits = []
        for w in range(W):
            l = (parts[w] + rolled[w][0]) + (rolled[w][1] + rolled[w][2])
            if first(t) and w > 0 and g * 8 < DIL * w:
                row = g * 8 + lax.broadcasted_iota(jnp.int32, (8, 128), 0)
                l = jnp.where(row >= DIL * w, l, MASKED2)
            logits.append(l)
        m = jnp.maximum(jnp.maximum(jnp.maximum(logits[0], logits[1]), jnp.maximum(logits[2], logits[3])),
                        jnp.maximum(jnp.maximum(logits[4], logits[5]), jnp.maximum(logits[6], logits[7])))
        pw = [jnp.exp2(l - m) for l in logits]
        den = ((pw[0] + pw[1]) + (pw[2] + pw[3])) + ((pw[4] + pw[5]) + (pw[6] + pw[7]))
        sums[(t[1], g)] = den
        inv = _recip(den)
        outs = []
        for j in range(4):
            acc = None
            for w in range(W):
                pr = pw[w] * v_scr[j, rows(t, g * 8, 8, HALO - DIL * w), :]
                acc = pr if acc is None else acc + pr
            outs.append(acc * inv)
        return outs

    def attn(t, m):
        c = t[1]
        if m < G:
            pending[(c, m)] = attn_logits(t, m)
        g = m - LAG
        if g >= 0:
            pending[(c, g, "o")] = attn_values(t, g, pending.pop((c, g)))
            if g % 2 == 1:
                a, b = pending.pop((c, g - 1, "o")), pending.pop((c, g, "o"))
                for j in range(4):
                    o_scr[j, rows(t, (g - 1) * 8, 16), :] = jnp.concatenate([a[j], b[j]], axis=0).astype(BF)

    def proj(t, jn):
        lhs = jnp.concatenate([_as_bf16(ow[kk, wrows(t, 0, TM), :]) for kk in range(4)], axis=1)
        res = jnp.dot(lhs, _as_bf16(wop32[jn]), preferred_element_type=F32)
        seen["proj", t[1], jn] = res[0:8, :]
        h_scr[jn, rows(t, 0, TM), :] = res + x_vm[rows(t, 0, TM), jn * 128:(jn + 1) * 128].astype(F32)

    def ln2(t):
        for r in range(0, TM, 16):
            y = _layernorm([h_scr[jn, rows(t, r, 16), :] for jn in range(4)])
            for kk in range(4):
                hln[kk, rows(t, r, 16), :] = y[kk].astype(BF)

    def up(t, j):
        lhs = jnp.concatenate([_as_bf16(hlnw[kk, wrows(t, 0, TM), :]) for kk in range(4)], axis=1)
        rhs = jnp.concatenate([_as_bf16(w1w[kk, j * 64:(j + 1) * 64, :]) for kk in range(4)], axis=1)
        pre = lax.dot_general(lhs, rhs, NT_DIMS, preferred_element_type=F32)
        pre = pre + jnp.tile(b1_scr[j], (TM // 8, 1))
        e = jnp.exp(jnp.minimum(pre, 20.0))
        n = e * (e + 2.0)
        den = n + 2.0
        gates[j] = den[0:8, :]
        act[j, rows(t, 0, TM), :] = (pre * n * _recip(den)).astype(BF)

    def down(t, jn):
        lhs = jnp.concatenate([_as_bf16(actw[j, wrows(t, 0, TM), :]) for j in range(NF)], axis=1)
        res = jnp.dot(lhs, _as_bf16(w2w[jn]), preferred_element_type=F32)
        out_vm[rows(t, 0, TM), jn * 128:(jn + 1) * 128] = (res + h_scr[jn, rows(t, 0, TM), :]).astype(BF)

    def out_tile(t):
        return cp(out_vm.at[rows(t, 0, TM), :], o_hbm.at[0, rows(t, 0, TM), :], OUT_SEM)

    def out_cols(t, jn):
        return cp(out_vm.at[rows(t, 0, TM), pl.ds(jn * 128, 128)], o_hbm.at[0, rows(t, 0, TM), pl.ds(jn * 128, 128)], OUT_SEM)

    def each(fn, t, lo, hi):
        return [lambda i=i: fn(t, i) for i in range(lo, hi + 1)]

    def run(thunks):
        for th in thunks:
            th()

    def weave(a, b):
        run(_weave(a, b))

    LAST = G + LAG - 1
    T = [(None, i) for i in range(NT)]

    start("x0", "qa", "qb", "x1", "b1", "k", "v")
    wait("x0", "qa")
    ln1(T[0])
    prep_q(0)
    wait("qb", z=after(seen["ln1", 0]))
    prep_q(1)
    wait("x1", "b1", z=after(seen["wq"]))
    ln1(T[1])
    run(each(qkv, T[0], 0, 3))
    wait("k", z=after(seen["qkv", 0, 3]))
    start("wo", "x2", z=after(seen["qkv", 0, 3]))
    prep_kv(0)
    run(each(qkv, T[1], 0, 3))
    run(each(qkv, T[0], 4, 4))
    wait("v", z=after(seen["qkv", 0, 4]))
    start("w1", z=after(seen["qkv", 0, 4]))
    prep_kv(1)
    run(each(qkv, T[0], 5, 7))
    run(each(qkv, T[1], 4, 4))
    run(each(qkv, T[0], 8, 11))
    wait("wo", "x2", z=after(seen["qkv", 0, 9]))
    start("w2", "xr", z=after(seen["qkv", 0, 9]))
    prep_wo()
    prep_b1()
    ln1(T[2])
    weave(each(qkv, T[1], 5, 11), each(attn, T[0], 0, LAST))
    run(each(proj, T[0], 0, 3))
    run(each(qkv, T[2], 0, 3))
    ln2(T[0])
    wait("w1", z=after(seen["proj", 0, 1]))
    run(each(up, T[0], 0, NF - 1))
    weave(each(qkv, T[2], 4, 7), each(attn, T[1], 0, 6))
    wait("w2", "xr", z=after(seen["qkv", 2, 4]))
    weave(each(qkv, T[2], 8, 11), each(attn, T[1], 7, 14))
    weave(each(down, T[0], 0, 3), each(attn, T[1], 15, LAST))
    ln1(T[3])
    out_tile(T[0]).start()

    def step(r, carry):
        sums.clear(); gates.clear(); pending.clear()
        s = 1 + r
        base = (pl.multiple_of(s * TM, TM), pl.multiple_of(s * (TM // 2), TM // 2))
        t0, t1, t2, t3 = (base, 0), (base, 1), (base, 2), (base, 3)
        run(each(proj, t0, 0, 3))
        run(each(qkv, t2, 0, 3))
        ln2(t0)
        run(each(up, t0, 0, NF - 1))
        weave(each(qkv, t2, 4, 11), each(attn, t1, 0, 14))
        weave(each(down, t0, 0, 3), each(attn, t1, 15, LAST))
        ln1(t3)
        out_tile(t0).start()
        sums.clear(); gates.clear(); pending.clear()
        return carry

    lax.fori_loop(0, 4, step, 0)

    run(each(proj, T[5], 0, 3))
    run(each(qkv, T[7], 0, 3))
    ln2(T[5])
    run(each(up, T[5], 0, NF - 1))
    weave(each(qkv, T[7], 4, 7), each(attn, T[6], 0, 7))
    weave(each(down, T[5], 0, 3), each(attn, T[6], 8, LAST))
    out_tile(T[5]).start()

    run(each(proj, T[6], 0, 3))
    run(each(qkv, T[7], 8, 11))
    ln2(T[6])
    run(each(up, T[6], 0, NF - 1))
    gates["on"] = NF - 1
    weave(each(down, T[6], 0, 2), each(attn, T[7], 0, LAST))
    gates["on"] = None

    run(each(proj, T[7], 0, 3))
    down(T[6], 3)
    ln2(T[7])
    out_tile(T[6]).start()
    run(each(up, T[7], 0, NF - 1))
    for jn in range(4):
        down(T[7], jn)
        out_cols(T[7], jn).start()

    for i in range(NT - 1):
        out_tile(T[i]).wait()
    for jn in range(4):
        out_cols(T[7], jn).wait()


@jax.jit
def pallas_sequential_preLN__sliding_local_dilated__dense_activation_mish__prompt_kernel(
    A_x: jax.Array,
    A_wqkv: jax.Array,
    A_wo: jax.Array,
    B_x: jax.Array,
    B_w1: jax.Array,
    B_b1: jax.Array,
    B_w2: jax.Array,
):
    del B_x
    hbm = pl.BlockSpec(memory_space=pltpu.HBM)
    return pl.pallas_call(
        _kernel,
        in_specs=[hbm] * 6,
        out_specs=hbm,
        out_shape=jax.ShapeDtypeStruct((1, S, D), BF),
        scratch_shapes=[
            pltpu.VMEM((S, D), BF),
            pltpu.VMEM((D, D), BF),
            pltpu.VMEM((2, D // 2, D), U32),
            pltpu.VMEM((2, 2, D + 16, 128), U32),
            pltpu.VMEM((2, 4, D // 2, 128), U32),
            pltpu.VMEM((4, D // 2 + 16, 128), U32),
            pltpu.VMEM((4, D // 2, 128), U32),
            pltpu.VMEM((4, FP, 128), BF),
            pltpu.VMEM((4, FP, 128), BF),
            pltpu.VMEM((4, D, 128), BF),
            pltpu.VMEM((4, S, 128), BF),
            pltpu.VMEM((4, S, 128), F32),
            pltpu.VMEM((4, HALO + S, 128), F32),
            pltpu.VMEM((4, HALO + S, 128), F32),
            pltpu.VMEM((4, S, 128), BF),
            pltpu.VMEM((4, S, 128), F32),
            pltpu.VMEM((4, S, 128), BF),
            pltpu.VMEM((NF, S, 128), BF),
            pltpu.VMEM((S, D), BF),
            pltpu.VMEM((NF, 8, 128), F32),
            pltpu.VMEM((F,), BF),
            pltpu.SemaphoreType.DMA((5,)),
        ],
        compiler_params=pltpu.CompilerParams(
            vmem_limit_bytes=64 << 20,
            flags={"XLA_TPU_RESCHEDULE_DMA_DONES": True},
        ),
        name="preln_dilated_attn_mish_ffn",
    )(A_x, A_wqkv, A_wo, B_w1.T, B_b1, B_w2)
```
